```python
import os as _os
_os.environ.setdefault("JAX_PLATFORMS", "cpu")
import jax
import jax.numpy as jnp

def _softmax(x, axis=-1):
    return jax.nn.softmax(x, axis=axis)
def _gelu(x):
    return jax.nn.gelu(x, approximate=True)
def _silu(x):
    return jax.nn.silu(x)
def _sigmoid(x):
    return jax.nn.sigmoid(x)
def _layernorm(x, axis=-1, eps=1e-5):
    m = jnp.mean(x, axis=axis, keepdims=True)
    v = jnp.var(x, axis=axis, keepdims=True)
    return (x - m) / jnp.sqrt(v + eps)
def _scatter_add(tgt, idx, src, axis=0):
    return tgt.at[idx].add(src)
def _segment_sum(src, seg, n):
    return jax.ops.segment_sum(src, seg, n)
class _Rng:
    def __init__(self, key):
        self._k = key
    def _next(self):
        self._k, sub = jax.random.split(self._k)
        return sub
    def normal(self, shape):
        return jax.random.normal(self._next(), shape, dtype=jnp.bfloat16)
    def randint(self, lo, hi, shape):
        return jax.random.randint(self._next(), shape, lo, hi, dtype=jnp.int32)
    def uniform(self, shape, lo=0.0, hi=1.0):
        return jax.random.uniform(self._next(), shape, jnp.bfloat16, lo, hi)
    def permutation(self, n):
        return jax.random.permutation(self._next(), n)


kernel_name = 'sequential_preLN__linear_kernel_hedgehog__dense_activation_squared_relu__prompt'

def setup_inputs():
    _rng = _Rng(jax.random.key(int.from_bytes(__import__("os").urandom(4), "little")))
    _w = (lambda a: (lambda t: t.astype(jnp.bfloat16) if jnp.issubdtype(t.dtype, jnp.floating) else t)(jnp.asarray(a)))
    def _A_setup():
        B, S, D, H = 1, 2048, 512, 32
        Dh = D // H
        return {
            "x": _w((lambda *s: _rng.normal(s) * 0.05)(B, S, D)),
            "wqkv": _w((lambda *s: _rng.normal(s) * 0.2)(D, 3 * D)),
            "w_phi": _w((lambda *s: _rng.normal(s) * 0.2)(H, Dh, Dh) * (Dh ** -0.5)),
            "wo": _w((lambda *s: _rng.normal(s) * 0.05)(D, D)),
        }
    _A_in = _A_setup()

    def _B_setup():
        B, S, D, F = 1, 2048, 512, 1792
        return {
            "x": _w((lambda *s: _rng.normal(s) * 0.05)(B, S, D)),
            "w1": _w((lambda *s: _rng.normal(s) * 0.05)(D, F)),
            "b1": _w((lambda *s: _rng.normal(s) * 0.05)(F)),
            "w2": _w((lambda *s: _rng.normal(s) * 0.05)(F, D)),
            "b2": _w((lambda *s: _rng.normal(s) * 0.05)(D)),
        }
    _B_in = _B_setup()

    return {
        "A_x": _A_in["x"],
        "A_wqkv": _A_in["wqkv"],
        "A_w_phi": _A_in["w_phi"],
        "A_wo": _A_in["wo"],
        "B_x": _B_in["x"],
        "B_w1": _B_in["w1"],
        "B_b1": _B_in["b1"],
        "B_w2": _B_in["w2"],
        "B_b2": _B_in["b2"],
    }

def reference(A_x, A_wqkv, A_w_phi, A_wo, B_x, B_w1, B_b1, B_w2, B_b2):
    def _A_ref(x, wqkv, w_phi, wo):
        B, S, D = x.shape
        H = 32; Dh = D // H
        qkv = (lambda x, *d: x.transpose(*d))((x @ wqkv).reshape(B, S, 3, H, Dh), 2, 0, 3, 1, 4)
        q, k, v = qkv[0], qkv[1], qkv[2]
        pq = jnp.einsum("bhsd,hdf->bhsf", q, w_phi)
        pk = jnp.einsum("bhsd,hdf->bhsf", k, w_phi)
        phi_q = jnp.concatenate([_softmax(pq, axis=-1), _softmax(-pq, axis=-1)], axis=-1)
        phi_k = jnp.concatenate([_softmax(pk, axis=-1), _softmax(-pk, axis=-1)], axis=-1)
        kv = jnp.einsum("bhsf,bhsd->bhfd", phi_k, v)
        z  = jnp.einsum("bhsf->bhf", phi_k)
        num = jnp.einsum("bhqf,bhfd->bhqd", phi_q, kv)
        den = jnp.einsum("bhqf,bhf->bhq", phi_q, z)[..., None] + 1e-6
        o = num / den
        return (lambda x, *d: x.transpose(*d))(o, 0, 2, 1, 3).reshape(B, S, D) @ wo

    def _B_ref(x, w1, b1, w2, b2):
        h = jnp.einsum("bsd,df->bsf", x, w1) + b1
        zero = jnp.zeros_like(h)
        r = jnp.where(h > zero, h, zero)
        h = r * r
        out = jnp.einsum("bsf,fd->bsd", h, w2) + b2
        return out

    x = A_x
    h = x + _A_ref(_layernorm(x, axis=-1), A_wqkv, A_w_phi, A_wo)
    h2 = h + _B_ref(_layernorm(h, axis=-1), B_w1, B_b1, B_w2, B_b2)
    return h2
```

```python
import jax
import jax.numpy as jnp
from jax import lax
import jax.experimental.pallas as pl
import jax.experimental.pallas.tpu as pltpu

_NT = (((1,), (1,)), ((), ()))
_NN = (((1,), (0,)), ((), ()))


def _mm(a, b, dims):
    return lax.dot_general(a, b, dims, preferred_element_type=jnp.float32)


def _layernorm(x):
    m = jnp.mean(x, axis=-1, keepdims=True)
    d = x - m
    v = jnp.mean(d * d, axis=-1, keepdims=True)
    return d * lax.rsqrt(v + 1e-5)


@jax.jit
def pallas_sequential_preLN__linear_kernel_hedgehog__dense_activation_squared_relu__prompt_kernel(
    A_x: jax.Array,
    A_wqkv: jax.Array,
    A_w_phi: jax.Array,
    A_wo: jax.Array,
    B_x: jax.Array,
    B_w1: jax.Array,
    B_b1: jax.Array,
    B_w2: jax.Array,
    B_b2: jax.Array,
):
    del B_x
    B, S, D = A_x.shape
    H, DH, _ = A_w_phi.shape
    F = B_w1.shape[1]
    assert B == 1 and D == H * DH and DH == 16 and H % 8 == 0
    G = H // 8
    T = 256
    NT = S // T
    assert S % T == 0
    f32, bf16 = jnp.float32, jnp.bfloat16

    def kernel_function(
        x_hbm, wqkv_hbm, wphi_hbm, wo_hbm, w1_hbm, b1_hbm, w2_hbm, b2_hbm, out_hbm,
        x_v, wqkv_v, wphi_v, wo_v, w1_v, b1_v, w2_v, b2_v, out_v,
        wqkT_v, phiq_v, kv_v, z_v, kvT_v,
        sem_x, sem_w, sem_o,
    ):
        def x_copy(t):
            return pltpu.make_async_copy(
                x_hbm.at[pl.ds(t * T, T), :], x_v.at[pl.ds(t * T, T), :], sem_x.at[t])

        c_phi = pltpu.make_async_copy(wphi_hbm, wphi_v, sem_w.at[0])
        c_qkv = pltpu.make_async_copy(wqkv_hbm, wqkv_v, sem_w.at[1])
        c_wo = pltpu.make_async_copy(wo_hbm, wo_v, sem_w.at[2])
        c_w1 = pltpu.make_async_copy(w1_hbm, w1_v, sem_w.at[3])
        c_b1 = pltpu.make_async_copy(b1_hbm, b1_v, sem_w.at[4])
        c_w2 = pltpu.make_async_copy(w2_hbm, w2_v, sem_w.at[5])
        c_b2 = pltpu.make_async_copy(b2_hbm, b2_v, sem_w.at[6])

        c_phi.start()
        c_qkv.start()
        for t in range(NT):
            x_copy(t).start()
        c_wo.start()
        c_w1.start()
        c_b1.start()
        c_w2.start()
        c_b2.start()

        c_phi.wait()
        c_qkv.wait()
        row = lax.broadcasted_iota(jnp.int32, (128, 128), 0)
        col = lax.broadcasted_iota(jnp.int32, (128, 128), 1)
        r16 = lax.broadcasted_iota(jnp.int32, (128, DH), 0)
        c16 = lax.broadcasted_iota(jnp.int32, (128, DH), 1)
        expand = jnp.where(r16 // 8 == c16, 1.0, 0.0).astype(bf16)
        same_head = (row % 8) == (col // DH)
        for g in range(G):
            wp = wphi_v[pl.ds(8 * g, 8)].reshape(128, DH)
            bdT = _mm(expand, wp, _NT)
            bdT = jnp.where(same_head, bdT, 0.0).astype(bf16)
            for part in range(2):
                wblk = wqkv_v[:, pl.ds(part * D + 128 * g, 128)]
                wqkT_v[pl.ds(part * D + 128 * g, 128), :] = _mm(bdT, wblk, _NT).astype(bf16)

        kv_v[...] = jnp.zeros(kv_v.shape, f32)
        z_v[...] = jnp.zeros(z_v.shape, f32)

        def feat(p):
            mx = jnp.max(p, axis=0, keepdims=True)
            mn = jnp.min(p, axis=0, keepdims=True)
            ep = jnp.exp(p - mx)
            en = jnp.exp(mn - p)
            ep = ep * pl.reciprocal(jnp.sum(ep, axis=0, keepdims=True))
            en = en * pl.reciprocal(jnp.sum(en, axis=0, keepdims=True))
            return jnp.concatenate([ep, en], axis=0).reshape(256, T)

        def phase1(t, carry):
            r0 = pl.multiple_of(t * T, T)
            x_copy(t).wait()
            x = x_v[pl.ds(r0, T), :].astype(f32)
            xn = _layernorm(x).astype(bf16)
            pT = _mm(wqkT_v[...], xn, _NT)
            v = _mm(xn, wqkv_v[:, pl.ds(2 * D, D)], _NN).astype(bf16)
            for g in range(G):
                pq = pT[128 * g:128 * (g + 1)].reshape(DH, 8, T)
                phiq_v[g, :, pl.ds(r0, T)] = feat(pq).astype(bf16)
                pk = pT[D + 128 * g:D + 128 * (g + 1)].reshape(DH, 8, T)
                fk = feat(pk)
                zs = fk[:, 0:128]
                for j in range(1, T // 128):
                    zs = zs + fk[:, 128 * j:128 * (j + 1)]
                z_v[g] += zs
                kv_v[g] += _mm(fk.astype(bf16), v[:, 128 * g:128 * (g + 1)], _NN)
            return carry

        lax.fori_loop(0, NT, phase1, 0)

        r256 = lax.broadcasted_iota(jnp.int32, (256, 128), 0)
        c256 = lax.broadcasted_iota(jnp.int32, (256, 128), 1)
        kv_mask = (r256 % 8) == (c256 // DH)
        z_mask = (r256 % 8) == c256
        for g in range(G):
            kvm = jnp.where(kv_mask, kv_v[g], 0.0)
            z = jnp.sum(z_v[g], axis=-1, keepdims=True)
            zm = jnp.where(z_mask, z, 0.0)
            kvT_v[g, 0:128, :] = kvm.T.astype(bf16)
            kvT_v[g, 128:144, :] = zm.T[0:16].astype(bf16)

        c_wo.wait()
        c_w1.wait()
        c_b1.wait()
        c_w2.wait()
        c_b2.wait()

        def o_copy(t):
            return pltpu.make_async_copy(
                out_v.at[pl.ds(t * T, T), :], out_hbm.at[pl.ds(t * T, T), :], sem_o.at[t])

        def phase2(t, carry):
            r0 = pl.multiple_of(t * T, T)
            oT = []
            for g in range(G):
                nd = _mm(kvT_v[g], phiq_v[g, :, pl.ds(r0, T)], _NN)
                inv = pl.reciprocal(nd[128:136] + 1e-6)
                num = nd[0:128].reshape(8, DH, T)
                oT.append((num * inv.reshape(8, 1, T)).reshape(128, T))
            oT = jnp.concatenate(oT, axis=0)
            o = oT.T.astype(bf16)
            h = x_v[pl.ds(r0, T), :].astype(f32) + _mm(o, wo_v[...], _NN)
            hn = _layernorm(h).astype(bf16)
            a = _mm(hn, w1_v[...], _NN) + b1_v[...].astype(f32)
            a = jnp.maximum(a, 0.0)
            a = (a * a).astype(bf16)
            y = h + _mm(a, w2_v[...], _NN) + b2_v[...].astype(f32)
            out_v[pl.ds(r0, T), :] = y.astype(out_v.dtype)
            o_copy(t).start()
            return carry

        lax.fori_loop(0, NT, phase2, 0)
        for t in range(NT):
            o_copy(t).wait()

    any_spec = pl.BlockSpec(memory_space=pl.ANY)
    out = pl.pallas_call(
        kernel_function,
        out_shape=jax.ShapeDtypeStruct((S, D), A_x.dtype),
        in_specs=[any_spec] * 8,
        out_specs=any_spec,
        scratch_shapes=[
            pltpu.VMEM((S, D), A_x.dtype),
            pltpu.VMEM((D, 3 * D), A_wqkv.dtype),
            pltpu.VMEM((H, DH, DH), A_w_phi.dtype),
            pltpu.VMEM((D, D), A_wo.dtype),
            pltpu.VMEM((D, F), B_w1.dtype),
            pltpu.VMEM((1, F), B_b1.dtype),
            pltpu.VMEM((F, D), B_w2.dtype),
            pltpu.VMEM((1, D), B_b2.dtype),
            pltpu.VMEM((S, D), A_x.dtype),
            pltpu.VMEM((2 * D, D), bf16),
            pltpu.VMEM((G, 256, S), bf16),
            pltpu.VMEM((G, 256, 128), f32),
            pltpu.VMEM((G, 256, 128), f32),
            pltpu.VMEM((G, 144, 256), bf16),
            pltpu.SemaphoreType.DMA((NT,)),
            pltpu.SemaphoreType.DMA((7,)),
            pltpu.SemaphoreType.DMA((NT,)),
        ],
        compiler_params=pltpu.CompilerParams(vmem_limit_bytes=100 * 1024 * 1024),
    )(A_x.reshape(S, D), A_wqkv, A_w_phi, A_wo, B_w1, B_b1.reshape(1, F), B_w2,
      B_b2.reshape(1, D))
    return out.reshape(B, S, D)
```

```python
import jax
import jax.numpy as jnp
from jax import lax
import jax.experimental.pallas as pl
import jax.experimental.pallas.tpu as pltpu

_NT = (((1,), (1,)), ((), ()))
_NN = (((1,), (0,)), ((), ()))

T1 = 512
T2 = 512
OC = 128
WC = 128
RC = 128


_LOG2E = 1.4426950408889634


def _recip(s):
    r = pl.reciprocal(s, approx=True)
    return r * (2.0 - s * r)


def _layernorm(x):
    m = jnp.mean(x, axis=-1, keepdims=True)
    d = x - m
    v = jnp.mean(d * d, axis=-1, keepdims=True)
    return d * lax.rsqrt(v + 1e-5)


@jax.jit
def pallas_sequential_preLN__linear_kernel_hedgehog__dense_activation_squared_relu__prompt_kernel(
    A_x: jax.Array,
    A_wqkv: jax.Array,
    A_w_phi: jax.Array,
    A_wo: jax.Array,
    B_x: jax.Array,
    B_w1: jax.Array,
    B_b1: jax.Array,
    B_w2: jax.Array,
    B_b2: jax.Array,
):
    del B_x
    B, S, D = A_x.shape
    H, DH, _ = A_w_phi.shape
    F = B_w1.shape[1]
    assert B == 1 and D == H * DH and DH == 16 and H % 8 == 0
    G = H // 8
    N1 = S // T1
    N2 = S // T2
    NO = S // OC
    NC = T2 // OC
    f32, bf16 = jnp.float32, jnp.bfloat16

    def kernel_function(
        x_hbm, wqkv_hbm, wphi_hbm, wo_hbm, w1_hbm, b1_hbm, w2_hbm, b2_hbm, out_hbm,
        x_v, wqkv_v, wphi_v, wo_v, w1_v, b1_v, w2_v, b2_v, out_v,
        wqT_v, wkT_v, xn_v, phiq_v, kv_v, z_v, kvT_v, h_v, hn_v,
        sem_w, sem_o,
    ):
        def x_copy(t):
            return pltpu.make_async_copy(
                x_hbm.at[pl.ds(t * T1, T1), :], x_v.at[pl.ds(t * T1, T1), :], sem_w.at[9 + t])

        def w_part(p):
            return pltpu.make_async_copy(
                wqkv_hbm.at[:, pl.ds(p * D, D)], wqkv_v.at[:, pl.ds(p * D, D)], sem_w.at[p])

        c_phi = pltpu.make_async_copy(wphi_hbm, wphi_v, sem_w.at[3])
        c_wo = pltpu.make_async_copy(wo_hbm, wo_v, sem_w.at[4])
        c_w1 = pltpu.make_async_copy(w1_hbm, w1_v, sem_w.at[5])
        c_b1 = pltpu.make_async_copy(b1_hbm, b1_v, sem_w.at[6])
        c_w2 = pltpu.make_async_copy(w2_hbm, w2_v, sem_w.at[7])
        c_b2 = pltpu.make_async_copy(b2_hbm, b2_v, sem_w.at[8])

        HT = T1 // 2
        c_x0a = pltpu.make_async_copy(x_hbm.at[pl.ds(0, HT), :], x_v.at[pl.ds(0, HT), :], sem_w.at[9])
        c_x0b = pltpu.make_async_copy(x_hbm.at[pl.ds(HT, HT), :], x_v.at[pl.ds(HT, HT), :], sem_w.at[9 + N1])

        c_phi.start()
        c_x0a.start()
        w_part(1).start()
        c_x0b.start()
        w_part(2).start()
        x_copy(1).start()
        w_part(0).start()
        for t in range(2, N1):
            x_copy(t).start()
        c_wo.start()
        c_w1.start()
        c_b1.start()
        c_w2.start()
        c_b2.start()

        def ln_rows(src, dst, n):
            for r in range(n // RC):
                x = x_v[pl.ds(pl.multiple_of(src + r * RC, RC), RC), :].astype(f32)
                xn_v[pl.ds(pl.multiple_of(dst + r * RC, RC), RC), :] = _layernorm(x).astype(bf16)

        c_phi.wait()
        row = lax.broadcasted_iota(jnp.int32, (128, 128), 0)
        col = lax.broadcasted_iota(jnp.int32, (128, 128), 1)
        same_head = (row % 8) == (col // DH)
        eh = lax.broadcasted_iota(jnp.int32, (H, D), 0)
        ec = lax.broadcasted_iota(jnp.int32, (H, D), 1)
        spread = jnp.where(eh == ec // DH, 1.0, 0.0).astype(bf16)
        xw = lax.dot_general(wphi_v[...], spread, _NN, preferred_element_type=f32)
        dr = lax.broadcasted_iota(jnp.int32, (DH * DH, D), 0) // DH
        dc = lax.broadcasted_iota(jnp.int32, (DH * DH, D), 1) % DH
        zw = jnp.sum(jnp.where(dr == dc, xw, 0.0).reshape(DH, DH, D), axis=0)
        bdT = []
        for g in range(G):
            zg = zw[:, 128 * g:128 * (g + 1)]
            b = jnp.broadcast_to(zg.reshape(DH, 1, 128), (DH, 8, 128)).reshape(128, 128)
            bdT.append(jnp.where(same_head, b, 0.0).astype(bf16))

        def fold(part, dst):
            for g in range(G):
                wblk = wqkv_v[:, pl.ds(part * D + 128 * g, 128)]
                dst[pl.ds(128 * g, 128), :] = (lax.dot_general(
                    bdT[g], wblk, _NT, preferred_element_type=f32) * _LOG2E).astype(bf16)

        def feat(p):
            p = p.reshape(DH, 8, 128)
            mx = jnp.max(p, axis=0, keepdims=True)
            mn = jnp.min(p, axis=0, keepdims=True)
            ep = jnp.exp2(p - mx)
            en = jnp.exp2(mn - p)
            ep = ep * _recip(jnp.sum(ep, axis=0, keepdims=True))
            en = en * _recip(jnp.sum(en, axis=0, keepdims=True))
            return jnp.concatenate([ep, en], axis=0).reshape(256, 128)

        def xn_rows(r0, n):
            return xn_v[pl.ds(pl.multiple_of(r0, 128), n), :]

        def proj_T(wT_v, xn):
            return lax.dot_general(wT_v[...], xn, _NT, preferred_element_type=f32)

        def v_proj(xn):
            return lax.dot_general(xn, wqkv_v[:, pl.ds(2 * D, D)], _NN,
                                   preferred_element_type=f32).astype(bf16)

        def q_stage(t):
            pT = proj_T(wqT_v, xn_rows(t * T2, T2))
            for j in range(T2 // 128):
                for g in range(G):
                    phiq_v[g, :, 128 * j:128 * (j + 1)] = feat(
                        pT[128 * g:128 * (g + 1), 128 * j:128 * (j + 1)]).astype(bf16)

        def k_feat(pT):
            fk = [[None] * (T1 // 128) for _ in range(G)]
            zs = [None] * G
            for j in range(T1 // 128):
                for g in range(G):
                    f = feat(pT[128 * g:128 * (g + 1), 128 * j:128 * (j + 1)])
                    zs[g] = f if j == 0 else zs[g] + f
                    fk[g][j] = f.astype(bf16)
            return fk, zs

        def kv_acc(fk, zs, v, first):
            for g in range(G):
                kv = lax.dot_general(jnp.concatenate(fk[g], axis=1), v[:, 128 * g:128 * (g + 1)],
                                     _NN, preferred_element_type=f32)
                if first:
                    z_v[g] = zs[g]
                    kv_v[g] = kv
                else:
                    z_v[g] += zs[g]
                    kv_v[g] += kv

        c_x0a.wait()
        ln_rows(0, 0, HT)
        w_part(1).wait()
        fold(1, wkT_v)
        c_x0b.wait()
        ln_rows(HT, HT, HT)
        pk = jnp.concatenate([proj_T(wkT_v, xn_rows(h * HT, HT)) for h in range(2)], axis=1)
        fk, zs = k_feat(pk)
        w_part(2).wait()
        x_copy(1).wait()
        w_part(0).wait()
        v = v_proj(xn_rows(0, T1))
        fold(0, wqT_v)
        ln_rows(T1, T1, T1)
        kv_acc(fk, zs, v, True)

        def phase1(t, carry):
            @pl.when(t + 1 < N1)
            def _():
                x_copy(t + 1).wait()

            xn = xn_rows(t * T1, T1)
            fk, zs = k_feat(proj_T(wkT_v, xn))
            v = v_proj(xn)
            ln_rows(jnp.minimum(t + 1, N1 - 1) * T1, (t + 1) * T1, T1)
            kv_acc(fk, zs, v, False)
            return carry

        lax.fori_loop(1, N1, phase1, 0)

        c_wo.wait()
        c_w1.wait()
        c_b1.wait()
        c_w2.wait()
        c_b2.wait()

        r256 = lax.broadcasted_iota(jnp.int32, (256, 128), 0)
        c256 = lax.broadcasted_iota(jnp.int32, (256, 128), 1)
        kv_mask = (r256 % 8) == (c256 // DH)
        z_mask = (r256 % 8) == c256
        for g in range(G):
            kvm = jnp.where(kv_mask, kv_v[g], 0.0)
            z = jnp.sum(z_v[g], axis=-1, keepdims=True)
            zm = jnp.where(z_mask, z, 0.0)
            kvT_v[g, 0:128, :] = kvm.T.astype(bf16)
            kvT_v[g, 128:144, :] = zm.T[0:16].astype(bf16)

        q_stage(0)

        def num_stage():
            oT = []
            for g in range(G):
                nd = lax.dot_general(kvT_v[g], phiq_v[g], _NN,
                                     preferred_element_type=f32)
                inv = _recip(nd[128:136] + 1e-6)
                num = nd[0:128].reshape(8, DH, T2)
                oT.append((num * inv.reshape(8, 1, T2)).reshape(128, T2))
            oT = jnp.concatenate(oT, axis=0)
            return oT.T.astype(bf16)

        def wo_stage(t, o):
            for r in range(T2 // WC):
                a = lax.dot_general(o[r * WC:(r + 1) * WC], wo_v[...], _NN,
                                    preferred_element_type=f32)
                rows = pl.ds(pl.multiple_of(t * T2 + r * WC, WC), WC)
                h = x_v[rows, :].astype(f32) + a
                h_v[rows, :] = h
                hn_v[rows, :] = _layernorm(h).astype(bf16)

        def ffn1(t):
            hn = hn_v[pl.ds(pl.multiple_of(t * T2, T2), T2), :]
            a = lax.dot_general(hn, w1_v[...], _NN, preferred_element_type=f32)
            a = jnp.maximum(a + b1_v[...].astype(f32).reshape(1, F), 0.0)
            return (a * a).astype(bf16)

        def o_copy(c):
            return pltpu.make_async_copy(
                out_v.at[pl.ds(c * OC, OC), :], out_hbm.at[pl.ds(c * OC, OC), :], sem_o.at[c])

        def ffn2(t, a, lo, hi):
            for j in range(lo, hi):
                c = t * (T2 // OC) + j
                rows = pl.ds(pl.multiple_of(c * OC, OC), OC)
                y = lax.dot_general(a[j * OC:(j + 1) * OC], w2_v[...], _NN,
                                    preferred_element_type=f32)
                y = h_v[rows, :] + (y + b2_v[...].astype(f32).reshape(1, D))
                out_v[rows, :] = y.astype(out_v.dtype)
                o_copy(c).start()

        wo_stage(0, num_stage())

        def phase2(t, carry):
            q_stage(t + 1)
            a = ffn1(t)
            o = num_stage()
            ffn2(t, a, 0, NC // 2)
            wo_stage(t + 1, o)
            ffn2(t, a, NC // 2, NC)
            return carry

        lax.fori_loop(0, N2 - 1, phase2, 0)
        ffn2(N2 - 1, ffn1(N2 - 1), 0, NC)
        for c in range(NO):
            o_copy(c).wait()

    any_spec = pl.BlockSpec(memory_space=pl.ANY)
    out = pl.pallas_call(
        kernel_function,
        out_shape=jax.ShapeDtypeStruct((S, D), A_x.dtype),
        in_specs=[any_spec] * 8,
        out_specs=any_spec,
        scratch_shapes=[
            pltpu.VMEM((S, D), A_x.dtype),
            pltpu.VMEM((D, 3 * D), A_wqkv.dtype),
            pltpu.VMEM((DH * DH, H), A_w_phi.dtype),
            pltpu.VMEM((D, D), A_wo.dtype),
            pltpu.VMEM((D, F), B_w1.dtype),
            pltpu.VMEM((F,), B_b1.dtype),
            pltpu.VMEM((F, D), B_w2.dtype),
            pltpu.VMEM((D,), B_b2.dtype),
            pltpu.VMEM((S, D), A_x.dtype),
            pltpu.VMEM((D, D), bf16),
            pltpu.VMEM((D, D), bf16),
            pltpu.VMEM((S + T1, D), bf16),
            pltpu.VMEM((G, 256, T2), bf16),
            pltpu.VMEM((G, 256, 128), f32),
            pltpu.VMEM((G, 256, 128), f32),
            pltpu.VMEM((G, 144, 256), bf16),
            pltpu.VMEM((S, D), f32),
            pltpu.VMEM((S, D), bf16),
            pltpu.SemaphoreType.DMA((10 + N1,)),
            pltpu.SemaphoreType.DMA((NO,)),
        ],
        compiler_params=pltpu.CompilerParams(vmem_limit_bytes=100 * 1024 * 1024),
    )(A_x.reshape(S, D), A_wqkv, jnp.transpose(A_w_phi, (1, 2, 0)).reshape(DH * DH, H),
      A_wo, B_w1, B_b1, B_w2, B_b2)
    return out.reshape(B, S, D)
```

```python
import jax
import jax.numpy as jnp
from jax import lax
import jax.experimental.pallas as pl
import jax.experimental.pallas.tpu as pltpu

_NT = (((1,), (1,)), ((), ()))
_NN = (((1,), (0,)), ((), ()))

T1 = 512
T2 = 512
OC = 128
WC = 128
RC = 32


_LOG2E = 1.4426950408889634


def _recip(s):
    r = pltpu.reciprocal(s, approx=True)
    return r * (2.0 - s * r)


def _layernorm(x):
    m = jnp.mean(x, axis=-1, keepdims=True)
    d = x - m
    v = jnp.mean(d * d, axis=-1, keepdims=True)
    return d * jnp.exp2(-0.5 * jnp.log2(v + 1e-5))


@jax.jit
def pallas_sequential_preLN__linear_kernel_hedgehog__dense_activation_squared_relu__prompt_kernel(
    A_x: jax.Array,
    A_wqkv: jax.Array,
    A_w_phi: jax.Array,
    A_wo: jax.Array,
    B_x: jax.Array,
    B_w1: jax.Array,
    B_b1: jax.Array,
    B_w2: jax.Array,
    B_b2: jax.Array,
):
    del B_x
    B, S, D = A_x.shape
    H, DH, _ = A_w_phi.shape
    F = B_w1.shape[1]
    assert B == 1 and D == H * DH and DH == 16 and H % 8 == 0
    G = H // 8
    N1 = S // T1
    N2 = S // T2
    NO = S // OC
    NC = T2 // OC
    f32, bf16 = jnp.float32, jnp.bfloat16

    def kernel_function(
        x_hbm, wqkv_hbm, wphi_hbm, wo_hbm, w1_hbm, b1_hbm, w2_hbm, b2_hbm, out_hbm,
        x_v, wqkv_v, wphi_v, wo_v, w1_v, b1_v, w2_v, b2_v, out_v,
        wqT_v, wkT_v, wvT_v, xn_v, phiq_v, kv_v, kvT_v, h_v, hn_v,
        sem_w, sem_o,
    ):
        def x_copy(t):
            return pltpu.make_async_copy(
                x_hbm.at[pl.ds(t * T1, T1), :], x_v.at[pl.ds(t * T1, T1), :], sem_w.at[9 + t])

        def w_part(p):
            return pltpu.make_async_copy(
                wqkv_hbm.at[:, pl.ds(p * D, D)], wqkv_v.at[:, pl.ds(p * D, D)], sem_w.at[p])

        c_phi = pltpu.make_async_copy(wphi_hbm, wphi_v, sem_w.at[3])
        c_wo = pltpu.make_async_copy(wo_hbm, wo_v, sem_w.at[4])
        c_w1 = pltpu.make_async_copy(w1_hbm, w1_v, sem_w.at[5])
        c_b1 = pltpu.make_async_copy(b1_hbm, b1_v, sem_w.at[6])
        c_w2 = pltpu.make_async_copy(w2_hbm, w2_v, sem_w.at[7])
        c_b2 = pltpu.make_async_copy(b2_hbm, b2_v, sem_w.at[8])

        HT = T1 // 2
        c_x0a = pltpu.make_async_copy(x_hbm.at[pl.ds(0, HT), :], x_v.at[pl.ds(0, HT), :], sem_w.at[9])
        c_x0b = pltpu.make_async_copy(x_hbm.at[pl.ds(HT, HT), :], x_v.at[pl.ds(HT, HT), :], sem_w.at[9 + N1])

        c_phi.start()
        c_x0a.start()
        w_part(1).start()
        c_x0b.start()
        w_part(2).start()
        for t in range(1, N1):
            x_copy(t).start()
        w_part(0).start()
        c_wo.start()
        c_w1.start()
        c_b1.start()
        c_w2.start()
        c_b2.start()

        def ln_rows(src, dst, n):
            for r in range(n // RC):
                x = x_v[pl.ds(pl.multiple_of(src + r * RC, RC), RC), :].astype(f32)
                xn_v[pl.ds(pl.multiple_of(dst + r * RC, RC), RC), :] = _layernorm(x).astype(bf16)

        c_phi.wait()
        row = lax.broadcasted_iota(jnp.int32, (128, 128), 0)
        col = lax.broadcasted_iota(jnp.int32, (128, 128), 1)
        same_head = (row % 8) == (col // DH)
        eh = lax.broadcasted_iota(jnp.int32, (H, D), 0)
        ec = lax.broadcasted_iota(jnp.int32, (H, D), 1)
        spread = jnp.where(eh == ec // DH, 1.0, 0.0).astype(bf16)
        xw = lax.dot_general(wphi_v[...], spread, _NN, preferred_element_type=f32)
        dr = lax.broadcasted_iota(jnp.int32, (DH * DH, D), 0) // DH
        dc = lax.broadcasted_iota(jnp.int32, (DH * DH, D), 1) % DH
        zw = jnp.sum(jnp.where(dr == dc, xw, 0.0).reshape(DH, DH, D), axis=0)
        bdT = []
        for g in range(G):
            zg = zw[:, 128 * g:128 * (g + 1)]
            b = jnp.broadcast_to(zg.reshape(DH, 1, 128), (DH, 8, 128)).reshape(128, 128)
            bdT.append(jnp.where(same_head, b, 0.0).astype(bf16))

        def fold(part, dst):
            for g in range(G):
                wblk = wqkv_v[:, pl.ds(part * D + 128 * g, 128)]
                dst[pl.ds(128 * g, 128), :] = (lax.dot_general(
                    bdT[g], wblk, _NT, preferred_element_type=f32) * _LOG2E).astype(bf16)

        def feat(p):
            p = p.reshape(DH, 8, 128)
            mx = jnp.max(p, axis=0, keepdims=True)
            mn = jnp.min(p, axis=0, keepdims=True)
            ep = jnp.exp2(p - mx)
            en = jnp.exp2(mn - p)
            ep = ep * _recip(jnp.sum(ep, axis=0, keepdims=True))
            en = en * _recip(jnp.sum(en, axis=0, keepdims=True))
            return ep, en

        def regroup(ep, en):
            lo = lax.broadcasted_iota(jnp.int32, ep.shape, 1) < 4
            r = pltpu.roll(jnp.where(lo, en, ep), 4, 1)
            return jnp.where(lo, ep, r), jnp.where(lo, r, en)

        def xn_rows(r0, n):
            return xn_v[pl.ds(pl.multiple_of(r0, 128), n), :]

        def proj_T(wT_v, xn):
            return lax.dot_general(wT_v[...], xn, _NT, preferred_element_type=f32)

        def v_proj(xn):
            return proj_T(wvT_v, xn).astype(bf16)

        def q_stage(t):
            pT = proj_T(wqT_v, xn_rows(t * T2, T2))
            for j in range(T2 // 128):
                for g in range(G):
                    a, b = regroup(*feat(pT[128 * g:128 * (g + 1), 128 * j:128 * (j + 1)]))
                    phiq_v[g, :, 128 * j:128 * (j + 1)] = jnp.concatenate(
                        [a, b], axis=0).reshape(256, 128).astype(bf16)

        def k_feat(pT):
            out = [[[None] * (T1 // 128) for _ in range(2)] for _ in range(G)]
            for j in range(T1 // 128):
                for g in range(G):
                    ab = regroup(*feat(pT[128 * g:128 * (g + 1), 128 * j:128 * (j + 1)]))
                    for hf in range(2):
                        out[g][hf][j] = ab[hf].reshape(128, 128).astype(bf16)
            return out

        def kv_acc(fk, vT, first):
            ones = jnp.ones((16, T1), bf16)
            for g in range(G):
                for hf in range(2):
                    r0 = 128 * g + 64 * hf
                    kv = lax.dot_general(
                        jnp.concatenate([vT[r0:r0 + 64], ones], axis=0),
                        jnp.concatenate(fk[g][hf], axis=1), _NT, preferred_element_type=f32)
                    if first:
                        kv_v[g, hf] = kv
                    else:
                        kv_v[g, hf] += kv

        c_x0a.wait()
        ln_rows(0, 0, HT)
        w_part(1).wait()
        fold(1, wkT_v)
        c_x0b.wait()
        ln_rows(HT, HT, HT)
        pk = jnp.concatenate([proj_T(wkT_v, xn_rows(h * HT, HT)) for h in range(2)], axis=1)
        fk = k_feat(pk)
        w_part(2).wait()
        x_copy(1).wait()
        for g in range(G):
            wvT_v[pl.ds(128 * g, 128), :] = wqkv_v[:, pl.ds(2 * D + 128 * g, 128)].T
        v = v_proj(xn_rows(0, T1))
        ln_rows(T1, T1, T1)
        kv_acc(fk, v, True)

        def phase1(t, carry):
            @pl.when(t + 1 < N1)
            def _():
                x_copy(t + 1).wait()

            xn = xn_rows(t * T1, T1)
            fk = k_feat(proj_T(wkT_v, xn))
            v = v_proj(xn)
            ln_rows(jnp.minimum(t + 1, N1 - 1) * T1, (t + 1) * T1, T1)
            kv_acc(fk, v, False)
            return carry

        lax.fori_loop(1, N1, phase1, 0)

        w_part(0).wait()
        c_wo.wait()
        c_w1.wait()
        c_b1.wait()
        c_w2.wait()
        c_b2.wait()

        r80 = lax.broadcasted_iota(jnp.int32, (80, 128), 0)
        c80 = lax.broadcasted_iota(jnp.int32, (80, 128), 1)
        kv_mask = jnp.where(r80 < 64, r80 // DH, r80 - 64) == (c80 % 4)
        for g in range(G):
            for hf in range(2):
                kvT_v[g, hf] = jnp.where(kv_mask, kv_v[g, hf], 0.0).astype(bf16)

        fold(0, wqT_v)
        q_stage(0)

        def num_stage():
            oT = []
            for g in range(G):
              for hf in range(2):
                nd = lax.dot_general(kvT_v[g, hf], phiq_v[g, 128 * hf:128 * (hf + 1), :], _NN,
                                     preferred_element_type=f32)
                inv = _recip(nd[64:72] + 1e-6)
                num = nd[0:64].reshape(4, DH, T2)
                oT.append((num * inv[0:4].reshape(4, 1, T2)).reshape(64, T2))
            oT = jnp.concatenate(oT, axis=0)
            return oT.T.astype(bf16)

        def wo_stage(t, o):
            for r in range(T2 // WC):
                a = lax.dot_general(o[r * WC:(r + 1) * WC], wo_v[...], _NN,
                                    preferred_element_type=f32)
                for u in range(WC // RC):
                    rows = pl.ds(pl.multiple_of(t * T2 + r * WC + u * RC, RC), RC)
                    h = x_v[rows, :].astype(f32) + a[u * RC:(u + 1) * RC]
                    h_v[rows, :] = h
                    hn_v[rows, :] = _layernorm(h).astype(bf16)

        def ffn1(t):
            hn = hn_v[pl.ds(pl.multiple_of(t * T2, T2), T2), :]
            a = lax.dot_general(hn, w1_v[...], _NN, preferred_element_type=f32)
            a = jnp.maximum(a + b1_v[...].astype(f32).reshape(1, F), 0.0)
            return (a * a).astype(bf16)

        def o_copy(c):
            return pltpu.make_async_copy(
                out_v.at[pl.ds(c * OC, OC), :], out_hbm.at[pl.ds(c * OC, OC), :], sem_o.at[c])

        def ffn2(t, a, lo, hi):
            for j in range(lo, hi):
                c = t * (T2 // OC) + j
                rows = pl.ds(pl.multiple_of(c * OC, OC), OC)
                y = lax.dot_general(a[j * OC:(j + 1) * OC], w2_v[...], _NN,
                                    preferred_element_type=f32)
                y = h_v[rows, :] + (y + b2_v[...].astype(f32).reshape(1, D))
                out_v[rows, :] = y.astype(out_v.dtype)
                o_copy(c).start()

        wo_stage(0, num_stage())

        def phase2(t, carry):
            q_stage(t + 1)
            a = ffn1(t)
            o = num_stage()
            ffn2(t, a, 0, NC // 2)
            wo_stage(t + 1, o)
            ffn2(t, a, NC // 2, NC)
            return carry

        lax.fori_loop(0, N2 - 1, phase2, 0)
        ffn2(N2 - 1, ffn1(N2 - 1), 0, NC)
        for c in range(NO):
            o_copy(c).wait()

    any_spec = pl.BlockSpec(memory_space=pl.ANY)
    out = pl.pallas_call(
        kernel_function,
        out_shape=jax.ShapeDtypeStruct((S, D), A_x.dtype),
        in_specs=[any_spec] * 8,
        out_specs=any_spec,
        scratch_shapes=[
            pltpu.VMEM((S, D), A_x.dtype),
            pltpu.VMEM((D, 3 * D), A_wqkv.dtype),
            pltpu.VMEM((DH * DH, H), A_w_phi.dtype),
            pltpu.VMEM((D, D), A_wo.dtype),
            pltpu.VMEM((D, F), B_w1.dtype),
            pltpu.VMEM((F,), B_b1.dtype),
            pltpu.VMEM((F, D), B_w2.dtype),
            pltpu.VMEM((D,), B_b2.dtype),
            pltpu.VMEM((S, D), A_x.dtype),
            pltpu.VMEM((D, D), bf16),
            pltpu.VMEM((D, D), bf16),
            pltpu.VMEM((D, D), bf16),
            pltpu.VMEM((S + T1, D), bf16),
            pltpu.VMEM((G, 256, T2), bf16),
            pltpu.VMEM((G, 2, 80, 128), f32),
            pltpu.VMEM((G, 2, 80, 128), bf16),
            pltpu.VMEM((S, D), f32),
            pltpu.VMEM((S, D), bf16),
            pltpu.SemaphoreType.DMA((10 + N1,)),
            pltpu.SemaphoreType.DMA((NO,)),
        ],
        compiler_params=pltpu.CompilerParams(vmem_limit_bytes=100 * 1024 * 1024),
    )(A_x.reshape(S, D), A_wqkv, jnp.transpose(A_w_phi, (1, 2, 0)).reshape(DH * DH, H),
      A_wo, B_w1, B_b1, B_w2, B_b2)
    return out.reshape(B, S, D)
```

```python
import jax
import jax.numpy as jnp
from jax import lax
import jax.experimental.pallas as pl
import jax.experimental.pallas.tpu as pltpu

_NT = (((1,), (1,)), ((), ()))
_NN = (((1,), (0,)), ((), ()))

T1 = 512
T2 = 512
OC = 128
WC = 128
RC = 32


_LOG2E = 1.4426950408889634


def _recip(s):
    r = pltpu.reciprocal(s, approx=True)
    return r * (2.0 - s * r)


def _layernorm(x):
    m = jnp.mean(x, axis=-1, keepdims=True)
    d = x - m
    v = jnp.mean(d * d, axis=-1, keepdims=True)
    return d * jnp.exp2(-0.5 * jnp.log2(v + 1e-5))


@jax.jit
def pallas_sequential_preLN__linear_kernel_hedgehog__dense_activation_squared_relu__prompt_kernel(
    A_x: jax.Array,
    A_wqkv: jax.Array,
    A_w_phi: jax.Array,
    A_wo: jax.Array,
    B_x: jax.Array,
    B_w1: jax.Array,
    B_b1: jax.Array,
    B_w2: jax.Array,
    B_b2: jax.Array,
):
    del B_x
    B, S, D = A_x.shape
    H, DH, _ = A_w_phi.shape
    F = B_w1.shape[1]
    assert B == 1 and D == H * DH and DH == 16 and H % 8 == 0
    G = H // 8
    N1 = S // T1
    N2 = S // T2
    NO = S // OC
    NC = T2 // OC
    f32, bf16 = jnp.float32, jnp.bfloat16

    def kernel_function(
        x_hbm, wqkv_hbm, wphi_hbm, wo_hbm, w1_hbm, b1_hbm, w2_hbm, b2_hbm, out_hbm,
        x_v, wqkv_v, wphi_v, wo_v, w1_v, b1_v, w2_v, b2_v, out_v,
        wqT_v, wkT_v, wvT_v, xn_v, phiq_v, kv_v, kvT_v, h_v, hn_v,
        sem_w, sem_o,
    ):
        def x_copy(t):
            return pltpu.make_async_copy(
                x_hbm.at[pl.ds(t * T1, T1), :], x_v.at[pl.ds(t * T1, T1), :], sem_w.at[9 + t])

        def w_part(p):
            return pltpu.make_async_copy(
                wqkv_hbm.at[:, pl.ds(p * D, D)], wqkv_v.at[:, pl.ds(p * D, D)], sem_w.at[p])

        c_phi = pltpu.make_async_copy(wphi_hbm, wphi_v, sem_w.at[3])
        c_wo = pltpu.make_async_copy(wo_hbm, wo_v, sem_w.at[4])
        c_w1 = pltpu.make_async_copy(w1_hbm, w1_v, sem_w.at[5])
        c_b1 = pltpu.make_async_copy(b1_hbm, b1_v, sem_w.at[6])
        c_w2 = pltpu.make_async_copy(w2_hbm, w2_v, sem_w.at[7])
        c_b2 = pltpu.make_async_copy(b2_hbm, b2_v, sem_w.at[8])

        HT = T1 // 2
        c_x0a = pltpu.make_async_copy(x_hbm.at[pl.ds(0, HT), :], x_v.at[pl.ds(0, HT), :], sem_w.at[9])
        c_x0b = pltpu.make_async_copy(x_hbm.at[pl.ds(HT, HT), :], x_v.at[pl.ds(HT, HT), :], sem_w.at[9 + N1])

        c_phi.start()
        c_x0a.start()
        w_part(1).start()
        c_x0b.start()
        w_part(2).start()
        for t in range(1, N1):
            x_copy(t).start()
        w_part(0).start()
        c_wo.start()
        c_w1.start()
        c_b1.start()
        c_w2.start()
        c_b2.start()

        def ln_rows(src, dst, n):
            for r in range(n // RC):
                x = x_v[pl.ds(pl.multiple_of(src + r * RC, RC), RC), :].astype(f32)
                xn_v[pl.ds(pl.multiple_of(dst + r * RC, RC), RC), :] = _layernorm(x).astype(bf16)

        c_phi.wait()
        row = lax.broadcasted_iota(jnp.int32, (128, 128), 0)
        col = lax.broadcasted_iota(jnp.int32, (128, 128), 1)
        same_head = (row % 8) == (col // DH)
        eh = lax.broadcasted_iota(jnp.int32, (H, D), 0)
        ec = lax.broadcasted_iota(jnp.int32, (H, D), 1)
        spread = jnp.where(eh == ec // DH, 1.0, 0.0).astype(bf16)
        xw = lax.dot_general(wphi_v[...], spread, _NN, preferred_element_type=f32)
        dr = lax.broadcasted_iota(jnp.int32, (DH * DH, D), 0) // DH
        dc = lax.broadcasted_iota(jnp.int32, (DH * DH, D), 1) % DH
        zw = jnp.sum(jnp.where(dr == dc, xw, 0.0).reshape(DH, DH, D), axis=0)
        bdT = []
        for g in range(G):
            zg = zw[:, 128 * g:128 * (g + 1)]
            b = jnp.broadcast_to(zg.reshape(DH, 1, 128), (DH, 8, 128)).reshape(128, 128)
            bdT.append(jnp.where(same_head, b, 0.0).astype(bf16))

        def fold(part, dst):
            for g in range(G):
                wblk = wqkv_v[:, pl.ds(part * D + 128 * g, 128)]
                dst[pl.ds(128 * g, 128), :] = (lax.dot_general(
                    bdT[g], wblk, _NT, preferred_element_type=f32) * _LOG2E).astype(bf16)

        def feat(p):
            p = p.reshape(DH, 8, 128)
            mx = jnp.max(p, axis=0, keepdims=True)
            mn = jnp.min(p, axis=0, keepdims=True)
            ep = jnp.exp2(p - mx)
            en = jnp.exp2(mn - p)
            ep = ep * _recip(jnp.sum(ep, axis=0, keepdims=True))
            en = en * _recip(jnp.sum(en, axis=0, keepdims=True))
            return ep, en

        def regroup(ep, en):
            lo = lax.broadcasted_iota(jnp.int32, ep.shape, 1) < 4
            r = pltpu.roll(jnp.where(lo, en, ep), 4, 1)
            return jnp.where(lo, ep, r), jnp.where(lo, r, en)

        def xn_rows(r0, n):
            return xn_v[pl.ds(pl.multiple_of(r0, 128), n), :]

        def proj_T(wT_v, xn):
            return lax.dot_general(wT_v[...], xn, _NT, preferred_element_type=f32)

        def v_proj(xn):
            return proj_T(wvT_v, xn).astype(bf16)

        def q_stage(t):
            pT = proj_T(wqT_v, xn_rows(t * T2, T2))
            for j in range(T2 // 128):
                for g in range(G):
                    a, b = regroup(*feat(pT[128 * g:128 * (g + 1), 128 * j:128 * (j + 1)]))
                    phiq_v[g, :, 128 * j:128 * (j + 1)] = jnp.concatenate(
                        [a, b], axis=0).reshape(256, 128).astype(bf16)

        def k_feat(pT):
            out = [[[None] * (T1 // 128) for _ in range(2)] for _ in range(G)]
            for j in range(T1 // 128):
                for g in range(G):
                    ab = regroup(*feat(pT[128 * g:128 * (g + 1), 128 * j:128 * (j + 1)]))
                    for hf in range(2):
                        out[g][hf][j] = ab[hf].reshape(128, 128).astype(bf16)
            return out

        def kv_acc(fk, vT, first):
            ones = jnp.ones((16, T1), bf16)
            for g in range(G):
                for hf in range(2):
                    r0 = 128 * g + 64 * hf
                    kv = lax.dot_general(
                        jnp.concatenate([vT[r0:r0 + 64], ones], axis=0),
                        jnp.concatenate(fk[g][hf], axis=1), _NT, preferred_element_type=f32)
                    if first:
                        kv_v[g, hf] = kv
                    else:
                        kv_v[g, hf] += kv

        c_x0a.wait()
        ln_rows(0, 0, HT)
        w_part(1).wait()
        fold(1, wkT_v)
        c_x0b.wait()
        ln_rows(HT, HT, HT)
        pk = jnp.concatenate([proj_T(wkT_v, xn_rows(h * HT, HT)) for h in range(2)], axis=1)
        fk = k_feat(pk)
        w_part(2).wait()
        x_copy(1).wait()
        for g in range(G):
            wvT_v[pl.ds(128 * g, 128), :] = wqkv_v[:, pl.ds(2 * D + 128 * g, 128)].T
        v = v_proj(xn_rows(0, T1))
        ln_rows(T1, T1, T1)
        kv_acc(fk, v, True)

        def phase1(t, carry):
            @pl.when(t + 1 < N1)
            def _():
                x_copy(t + 1).wait()

            xn = xn_rows(t * T1, T1)
            fk = k_feat(proj_T(wkT_v, xn))
            v = v_proj(xn)
            ln_rows(jnp.minimum(t + 1, N1 - 1) * T1, (t + 1) * T1, T1)
            kv_acc(fk, v, False)
            return carry

        lax.fori_loop(1, N1, phase1, 0)

        w_part(0).wait()
        c_wo.wait()
        c_w1.wait()
        c_b1.wait()
        c_w2.wait()
        c_b2.wait()

        r80 = lax.broadcasted_iota(jnp.int32, (80, 128), 0)
        c80 = lax.broadcasted_iota(jnp.int32, (80, 128), 1)
        kv_mask = jnp.where(r80 < 64, r80 // DH, r80 - 64) == (c80 % 4)
        for g in range(G):
            for hf in range(2):
                kvT_v[g, hf] = jnp.where(kv_mask, kv_v[g, hf], 0.0).astype(bf16)

        fold(0, wqT_v)
        q_stage(0)

        def num_stage():
            oT = []
            for g in range(G):
                for hf in range(2):
                    nd = lax.dot_general(kvT_v[g, hf], phiq_v[g, 128 * hf:128 * (hf + 1), :], _NN,
                                         preferred_element_type=f32)
                    inv = _recip(nd[64:72] + 1e-6)
                    num = nd[0:64].reshape(4, DH, T2)
                    oT.append((num * inv[0:4].reshape(4, 1, T2)).reshape(64, T2))
            oT = jnp.concatenate(oT, axis=0)
            return oT.T.astype(bf16)

        def wo_stage(t, o):
            for r in range(T2 // WC):
                a = lax.dot_general(o[r * WC:(r + 1) * WC], wo_v[...], _NN,
                                    preferred_element_type=f32)
                for u in range(WC // RC):
                    rows = pl.ds(pl.multiple_of(t * T2 + r * WC + u * RC, RC), RC)
                    h = x_v[rows, :].astype(f32) + a[u * RC:(u + 1) * RC]
                    h_v[rows, :] = h
                    hn_v[rows, :] = _layernorm(h).astype(bf16)

        def ffn1(t):
            hn = hn_v[pl.ds(pl.multiple_of(t * T2, T2), T2), :]
            a = lax.dot_general(hn, w1_v[...], _NN, preferred_element_type=f32)
            a = jnp.maximum(a + b1_v[...].astype(f32).reshape(1, F), 0.0)
            return (a * a).astype(bf16)

        def o_copy(c):
            return pltpu.make_async_copy(
                out_v.at[pl.ds(c * OC, OC), :], out_hbm.at[pl.ds(c * OC, OC), :], sem_o.at[c])

        def ffn2(t, a, lo, hi):
            for j in range(lo, hi):
                c = t * (T2 // OC) + j
                rows = pl.ds(pl.multiple_of(c * OC, OC), OC)
                y = lax.dot_general(a[j * OC:(j + 1) * OC], w2_v[...], _NN,
                                    preferred_element_type=f32)
                y = h_v[rows, :] + (y + b2_v[...].astype(f32).reshape(1, D))
                out_v[rows, :] = y.astype(out_v.dtype)
                o_copy(c).start()

        wo_stage(0, num_stage())

        def phase2(t, carry):
            q_stage(t + 1)
            a = ffn1(t)
            o = num_stage()
            ffn2(t, a, 0, NC // 2)
            wo_stage(t + 1, o)
            ffn2(t, a, NC // 2, NC)
            return carry

        lax.fori_loop(0, N2 - 1, phase2, 0)
        ffn2(N2 - 1, ffn1(N2 - 1), 0, NC)
        for c in range(NO):
            o_copy(c).wait()

    any_spec = pl.BlockSpec(memory_space=pl.ANY)
    out = pl.pallas_call(
        kernel_function,
        out_shape=jax.ShapeDtypeStruct((S, D), A_x.dtype),
        in_specs=[any_spec] * 8,
        out_specs=any_spec,
        scratch_shapes=[
            pltpu.VMEM((S, D), A_x.dtype),
            pltpu.VMEM((D, 3 * D), A_wqkv.dtype),
            pltpu.VMEM((DH * DH, H), A_w_phi.dtype),
            pltpu.VMEM((D, D), A_wo.dtype),
            pltpu.VMEM((D, F), B_w1.dtype),
            pltpu.VMEM((F,), B_b1.dtype),
            pltpu.VMEM((F, D), B_w2.dtype),
            pltpu.VMEM((D,), B_b2.dtype),
            pltpu.VMEM((S, D), A_x.dtype),
            pltpu.VMEM((D, D), bf16),
            pltpu.VMEM((D, D), bf16),
            pltpu.VMEM((D, D), bf16),
            pltpu.VMEM((S + T1, D), bf16),
            pltpu.VMEM((G, 256, T2), bf16),
            pltpu.VMEM((G, 2, 80, 128), f32),
            pltpu.VMEM((G, 2, 80, 128), bf16),
            pltpu.VMEM((S, D), f32),
            pltpu.VMEM((S, D), bf16),
            pltpu.SemaphoreType.DMA((10 + N1,)),
            pltpu.SemaphoreType.DMA((NO,)),
        ],
        compiler_params=pltpu.CompilerParams(vmem_limit_bytes=100 * 1024 * 1024),
    )(A_x.reshape(S, D), A_wqkv, jnp.transpose(A_w_phi, (1, 2, 0)).reshape(DH * DH, H),
      A_wo, B_w1, B_b1, B_w2, B_b2)
    return out.reshape(B, S, D)
```
